```python
import os as _os
_os.environ.setdefault('JAX_PLATFORMS', 'cpu')
import jax
import jax.numpy as jnp

def _softmax(x, axis=-1):
    return jax.nn.softmax(x, axis=axis)

def _gelu(x):
    return jax.nn.gelu(x, approximate=True)

def _silu(x):
    return jax.nn.silu(x)

def _sigmoid(x):
    return jax.nn.sigmoid(x)

def _layernorm(x, axis=-1, eps=1e-05):
    m = jnp.mean(x, axis=axis, keepdims=True)
    v = jnp.var(x, axis=axis, keepdims=True)
    return (x - m) / jnp.sqrt(v + eps)

def _scatter_add(tgt, idx, src, axis=0):
    return tgt.at[idx].add(src)

def _segment_sum(src, seg, n):
    return jax.ops.segment_sum(src, seg, n)

class _Rng:

    def __init__(self, key):
        self._k = key

    def _next(self):
        self._k, sub = jax.random.split(self._k)
        return sub

    def normal(self, shape):
        return jax.random.normal(self._next(), shape, dtype=jnp.bfloat16)

    def randint(self, lo, hi, shape):
        return jax.random.randint(self._next(), shape, lo, hi, dtype=jnp.int32)

    def uniform(self, shape, lo=0.0, hi=1.0):
        return jax.random.uniform(self._next(), shape, jnp.bfloat16, lo, hi)

    def permutation(self, n):
        return jax.random.permutation(self._next(), n)
kernel_name = 'sequential_preLN__linear_attn_block__mixer_gmlp__prompt'

def setup_inputs():
    _rng = _Rng(jax.random.key(int.from_bytes(__import__("os").urandom(4), "little")))
    _w = lambda a: (lambda t: t.astype(jnp.bfloat16) if jnp.issubdtype(t.dtype, jnp.floating) else t)(jnp.asarray(a))

    def _A_setup():
        B, S, D = (1, 2048, 512)
        return {'x': _w((lambda *s: _rng.normal(s) * 0.05)(B, S, D)), 'wqkv': _w((lambda *s: _rng.normal(s) * 0.05)(D, 3 * D)), 'wo': _w((lambda *s: _rng.normal(s) * 0.05)(D, D))}
    _A_in = _A_setup()

    def _B_setup():
        B, S, D, F = (1, 2048, 512, 1792)
        Fh = F // 2
        return {'x': _w((lambda *s: _rng.normal(s) * 0.05)(B, S, D)), 'w_in': _w((lambda *s: _rng.normal(s) * 0.4)(D, 2 * Fh)), 'w_sp': _w(0.01 * (lambda *s: _rng.normal(s) * 0.4)(S, S)), 'b_sp': _w(1.0 + 0.01 * (lambda *s: _rng.normal(s) * 0.05)(S)), 'w_out': _w((lambda *s: _rng.normal(s) * 0.05)(Fh, D))}
    _B_in = _B_setup()
    return {'A_x': _A_in['x'], 'A_wqkv': _A_in['wqkv'], 'A_wo': _A_in['wo'], 'B_x': _B_in['x'], 'B_w_in': _B_in['w_in'], 'B_w_sp': _B_in['w_sp'], 'B_b_sp': _B_in['b_sp'], 'B_w_out': _B_in['w_out']}

def reference(A_x, A_wqkv, A_wo, B_x, B_w_in, B_w_sp, B_b_sp, B_w_out):

    def _A_ref(x, wqkv, wo):
        B, S, D = x.shape
        H = 32
        Dh = D // H
        qkv = (lambda x, *d: x.transpose(*d))((x @ wqkv).reshape(B, S, 3, H, Dh), 2, 0, 3, 1, 4)
        q, k, v = (qkv[0], qkv[1], qkv[2])
        phi = lambda t: jnp.where(t > 0, t + 1, jnp.exp(t)) + 1e-06
        pq, pk = (phi(q), phi(k))
        kv = jnp.einsum('bhsd,bhse->bhde', pk, v)
        z = jnp.einsum('bhsd->bhd', pk)
        num = jnp.einsum('bhqd,bhde->bhqe', pq, kv)
        den = jnp.einsum('bhqd,bhd->bhq', pq, z)[..., None] + 1e-06
        o = num / den
        return (lambda x, *d: x.transpose(*d))(o, 0, 2, 1, 3).reshape(B, S, D) @ wo

    def _B_ref(x, w_in, w_sp, b_sp, w_out):
        B, S, D = x.shape
        F = w_in.shape[-1]
        Fh = F // 2
        z = _gelu(jnp.einsum('bsd,df->bsf', x, w_in))
        z1 = z[..., :Fh].copy()
        z2 = _layernorm(z[..., Fh:], axis=-1)
        g = jnp.einsum('ts,bsf->btf', w_sp, z2) + b_sp[None, :, None]
        return jnp.einsum('bsf,fd->bsd', z1 * g, w_out)
    x = A_x
    h = x + _A_ref(_layernorm(x, axis=-1), A_wqkv, A_wo)
    h2 = h + _B_ref(_layernorm(h, axis=-1), B_w_in, B_w_sp, B_b_sp, B_w_out)
    return h2
```

```python
import functools
import jax
import jax.numpy as jnp
from jax import lax
from jax.experimental import pallas as pl
from jax.experimental.pallas import tpu as pltpu

S, D, H, DH, FH = 2048, 512, 32, 16, 896
LN_EPS = 1e-5
F32, BF16 = jnp.float32, jnp.bfloat16
GELU_C = 0.7978845608028654


def _ln(xf):
    m = jnp.mean(xf, axis=-1, keepdims=True)
    xc = xf - m
    v = jnp.mean(xc * xc, axis=-1, keepdims=True)
    return xc * lax.rsqrt(v + LN_EPS)


def _phi(t):
    return jnp.where(t > 0, t + 1.0, jnp.exp(t)) + 1e-6


def _gelu(t):
    return (0.5 * t) * (1.0 + jnp.tanh(GELU_C * (t + 0.044715 * (t * t * t))))


def _kernel(x_hbm, wqkv_hbm, wo_hbm, win_hbm, wsp_hbm, b_hbm, wout_hbm, out_hbm,
            x_v, wqkv_v, wo_v, win_v, wsp_v, b_v, wout_v,
            pq_v, kv_v, zs_v, m_v, zbd_v, bb_v, h_v, z1_v, z2_v, o_v,
            sem_x, sem_w, sem_sp, sem_o, *, T1, T2, T3, phases):
    N1, N2, N3 = S // T1, S // T2, S // T3

    def x_copy(i):
        return pltpu.make_async_copy(x_hbm.at[0, pl.ds(i * T1, T1)], x_v.at[pl.ds(i * T1, T1)], sem_x.at[i])

    def sp_copy(i):
        return pltpu.make_async_copy(wsp_hbm.at[pl.ds(i * T3, T3)], wsp_v.at[pl.ds(i * T3, T3)], sem_sp.at[i])

    def o_copy(i):
        return pltpu.make_async_copy(o_v.at[pl.ds(i * T3, T3)], out_hbm.at[0, pl.ds(i * T3, T3)], sem_o.at[i])

    wqkv_copy = pltpu.make_async_copy(wqkv_hbm, wqkv_v, sem_w.at[0])
    wo_copy = pltpu.make_async_copy(wo_hbm, wo_v, sem_w.at[1])
    win_copy = pltpu.make_async_copy(win_hbm, win_v, sem_w.at[2])
    b_copy = pltpu.make_async_copy(b_hbm, b_v, sem_w.at[3])
    wout_copy = pltpu.make_async_copy(wout_hbm, wout_v, sem_w.at[4])

    x_copy(0).start()
    wqkv_copy.start()
    b_copy.start()
    for i in range(1, N1):
        x_copy(i).start()
    wo_copy.start()
    win_copy.start()

    b_copy.wait()
    for i in range(S // 128):
        row = b_v[pl.ds(i, 1), :].astype(F32)
        bb_v[pl.ds(i * 128, 128), :] = jnp.broadcast_to(row, (128, 128)).T

    kv_v[...] = jnp.zeros_like(kv_v)
    zs_v[...] = jnp.zeros_like(zs_v)
    wqkv_copy.wait()

    def p1(i, carry):
        x_copy(i).wait()
        r = pl.ds(pl.multiple_of(i * T1, T1), T1)
        xn = _ln(x_v[r, :].astype(F32)).astype(BF16)
        qkv = jnp.dot(xn, wqkv_v[...], preferred_element_type=F32)
        pq_v[r, :] = _phi(qkv[:, :D]).astype(BF16)
        pk = _phi(qkv[:, D:2 * D])
        zs_v[...] += jnp.sum(pk.reshape(T1 // 8, 8, D), axis=0)
        pkb = pk.astype(BF16)
        vb = qkv[:, 2 * D:].astype(BF16)
        for g in range(4):
            c = slice(g * 128, (g + 1) * 128)
            kv_v[g] += lax.dot_general(pkb[:, c], vb[:, c], (((0,), (0,)), ((), ())),
                                       preferred_element_type=F32)
        return carry

    with jax.named_scope("phase1"):
        lax.fori_loop(0, N1, p1, 0)

    for i in range(N3):
        sp_copy(i).start()
    wout_copy.start()

    wo_copy.wait()
    ri = lax.broadcasted_iota(jnp.int32, (128, 128), 0) // DH
    ci = lax.broadcasted_iota(jnp.int32, (128, 128), 1) // DH
    same = ri == ci
    zrow = jnp.sum(zs_v[...], axis=0, keepdims=True)
    for g in range(4):
        c = slice(g * 128, (g + 1) * 128)
        kvb = jnp.where(same, kv_v[g], 0.0).astype(BF16)
        m_v[g] = jnp.dot(kvb, wo_v[c, :], preferred_element_type=F32).astype(BF16)
        zcol = jnp.broadcast_to(zrow[:, c], (128, 128)).T
        zbd_v[g] = jnp.where(same, zcol, 0.0).astype(BF16)

    win_copy.wait()

    def p2(i, carry):
        r = pl.ds(pl.multiple_of(i * T2, T2), T2)
        acc = x_v[r, :].astype(F32)
        for g in range(4):
            c = slice(g * 128, (g + 1) * 128)
            pq = pq_v[r, c]
            den = jnp.dot(pq, zbd_v[g], preferred_element_type=F32) + 1e-6
            rr = (pq.astype(F32) / den).astype(BF16)
            acc = acc + jnp.dot(rr, m_v[g], preferred_element_type=F32)
        hb = acc.astype(BF16)
        h_v[r, :] = hb
        hn = _ln(hb.astype(F32)).astype(BF16)
        z = _gelu(jnp.dot(hn, win_v[...], preferred_element_type=F32))
        z1_v[r, :] = z[:, :FH].astype(BF16)
        z2_v[r, :] = _ln(z[:, FH:]).astype(BF16)
        return carry

    with jax.named_scope("phase2"):
        lax.fori_loop(0, N2, p2, 0)

    wout_copy.wait()

    def p3(i, carry):
        sp_copy(i).wait()
        r = pl.ds(pl.multiple_of(i * T3, T3), T3)
        g = jnp.dot(wsp_v[r, :], z2_v[...], preferred_element_type=F32)
        bb = bb_v[r, :]
        g = g + jnp.concatenate([bb] * (FH // 128), axis=1)
        y = (z1_v[r, :].astype(F32) * g).astype(BF16)
        o = jnp.dot(y, wout_v[...], preferred_element_type=F32) + h_v[r, :].astype(F32)
        o_v[r, :] = o.astype(BF16)
        o_copy(i).start()
        return carry

    with jax.named_scope("phase3"):
        lax.fori_loop(0, N3, p3, 0)

    for i in range(N3):
        o_copy(i).wait()


def make(T1=256, T2=256, T3=256, phases=3):
    @jax.jit
    def fn(A_x, A_wqkv, A_wo, B_x, B_w_in, B_w_sp, B_b_sp, B_w_out):
        del B_x
        any_spec = pl.BlockSpec(memory_space=pl.ANY)
        return pl.pallas_call(
            functools.partial(_kernel, T1=T1, T2=T2, T3=T3, phases=phases),
            in_specs=[any_spec] * 7,
            out_specs=any_spec,
            out_shape=jax.ShapeDtypeStruct((1, S, D), BF16),
            scratch_shapes=[
                pltpu.VMEM((S, D), BF16),
                pltpu.VMEM((D, 3 * D), BF16),
                pltpu.VMEM((D, D), BF16),
                pltpu.VMEM((D, 2 * FH), BF16),
                pltpu.VMEM((S, S), BF16),
                pltpu.VMEM((S // 128, 128), BF16),
                pltpu.VMEM((FH, D), BF16),
                pltpu.VMEM((S, D), BF16),
                pltpu.VMEM((4, 128, 128), F32),
                pltpu.VMEM((8, D), F32),
                pltpu.VMEM((4, 128, D), BF16),
                pltpu.VMEM((4, 128, 128), BF16),
                pltpu.VMEM((S, 128), F32),
                pltpu.VMEM((S, D), BF16),
                pltpu.VMEM((S, FH), BF16),
                pltpu.VMEM((S, FH), BF16),
                pltpu.VMEM((S, D), BF16),
                pltpu.SemaphoreType.DMA((S // T1,)),
                pltpu.SemaphoreType.DMA((5,)),
                pltpu.SemaphoreType.DMA((S // T3,)),
                pltpu.SemaphoreType.DMA((S // T3,)),
            ],
            compiler_params=pltpu.CompilerParams(vmem_limit_bytes=100 * 1024 * 1024),
        )(A_x, A_wqkv, A_wo, B_w_in, B_w_sp, B_b_sp.reshape(S // 128, 128), B_w_out)
    return fn


_fn = make(T1=512,T2=512,T3=512)


def pallas_sequential_preLN__linear_attn_block__mixer_gmlp__prompt_kernel(
        A_x, A_wqkv, A_wo, B_x, B_w_in, B_w_sp, B_b_sp, B_w_out):
    return _fn(A_x, A_wqkv, A_wo, B_x, B_w_in, B_w_sp, B_b_sp, B_w_out)
```

```python
import functools
import jax
import jax.numpy as jnp
from jax import lax
from jax.experimental import pallas as pl
from jax.experimental.pallas import tpu as pltpu

S, D, H, DH, FH = 2048, 512, 32, 16, 896
LN_EPS = 1e-5
F32, BF16, U32 = jnp.float32, jnp.bfloat16, jnp.uint32
GC1 = 0.7978845608028654
GC2 = GC1 * 0.044715
GA = GC2 ** (1.0 / 3.0)
GK = GC1 / GA
GS = 2.0 * GA
TN = (((0,), (0,)), ((), ()))


def _dot(a, b):
    return jnp.dot(a, b, preferred_element_type=F32)


def _ln(xf, n, s_in=1.0, s_out=1.0):
    m = jnp.sum(xf, axis=-1, keepdims=True) * (1.0 / n)
    xc = xf - m
    v = jnp.sum(xc * xc, axis=-1, keepdims=True) * (1.0 / (n * s_out * s_out))
    return xc * jnp.exp2(-0.5 * jnp.log2(v + LN_EPS * (s_in / s_out) ** 2))


def _phi(t):
    return (jnp.maximum(t, 0.0) + jnp.exp(jnp.minimum(t, 0.0))) + 1e-6


def _gelu2(t):
    return t + t * jnp.tanh(t * (t * t + GK))


def _cat(xs):
    return xs[0] if len(xs) == 1 else jnp.concatenate(xs, axis=1)


def _kernel(x_hbm, wqkv_hbm, wo_hbm, win_hbm, wsp_hbm, b_hbm, wout_hbm, out_hbm,
            x_v, wqkv_v, wo_v, win_v, wsp_v, b_v, wout_v,
            xn0, xn1, pq_v, a_v, zs_v, m_v, zbd_v, bb_v, h_v, hn0, hn1, z1_v, z2_v, z7_v, wos_v, wis_v, wqs_v, o_v, zt0, zt1,
            sem_x, sem_w, sem_sp, sem_o, *, T, T3, NCH, NCZ, ORD, SV, WO, GO, U2, U3, EO, WC, RF, KS, QS, QO, NCX):
    NB, N3 = S // T, S // T3
    QORD = ((0, 1, 2, 3, 4, 5, 6), (6, 0, 3, 4, 2, 1, 5), (3, 1, 4, 6, 0, 2, 5))[QO]
    EORD = ((0, 1, 2, 3, 4, 5, 6), (6, 0, 3, 4, 2, 1, 5), (3, 1, 4, 6, 0, 2, 5))[EO]
    GORD = ((0, 1, 2, 3, 4, 5, 6), (6, 0, 3, 4, 2, 1, 5), (3, 1, 4, 6, 0, 2, 5))[GO]
    T2 = T // 2

    def x_copy(i):
        return pltpu.make_async_copy(x_hbm.at[0, pl.ds(i * T, T)], x_v.at[pl.ds(i * T, T)], sem_x.at[i])

    def slab_copies(hbm, vm, lo, hi, sem):
        return [pltpu.make_async_copy(hbm.at[:, pl.ds(n * 128, 128)], vm.at[n], sem) for n in range(lo, hi)]

    def o_copy(i, n):
        return pltpu.make_async_copy(o_v.at[n, pl.ds(i * T3, T3)],
                                     out_hbm.at[0, pl.ds(i * T3, T3), pl.ds(n * 128, 128)], sem_o.at[i])

    wk_c = slab_copies(wqkv_hbm, wqkv_v, 4, 8, sem_w.at[0])
    wq_c = slab_copies(wqkv_hbm, wqkv_v, 0, 4, sem_w.at[1])
    wv_c = slab_copies(wqkv_hbm, wqkv_v, 8, 12, sem_w.at[2])
    wo_c = slab_copies(wo_hbm, wo_v, 0, 4, sem_w.at[3])
    win_c = slab_copies(win_hbm, win_v, 0, 14, sem_w.at[4])
    wout_c = slab_copies(wout_hbm, wout_v, 0, 4, sem_w.at[5])
    wsp_c = slab_copies(wsp_hbm, wsp_v, 0, 16, sem_sp.at[0])
    b_c = [pltpu.make_async_copy(b_hbm, b_v, sem_w.at[6])]

    def mo(v, m):
        return v if isinstance(v, int) else pl.multiple_of(v, m)

    def start(cs):
        for c in cs:
            c.start()

    def wait(cs):
        for c in cs:
            c.wait()

    def ldw(vm, n, r0=0, nr=None):
        v = vm.at[n].bitcast(U32)
        nr = v.shape[0] * 2 if nr is None else nr
        return pltpu.bitcast(v[pl.ds(r0 // 2, nr // 2), :], BF16)

    def ldp(ref, n, blk, tr=T2):
        r = blk * tr
        if not isinstance(blk, int):
            r = pl.multiple_of(r, tr)
        return pltpu.bitcast(ref.at[n].bitcast(U32)[pl.ds(r, tr), :], BF16)

    def stp(ref, n, blk, val, tr=T2):
        r = blk * (2 * tr)
        if not isinstance(blk, int):
            r = pl.multiple_of(r, 2 * tr)
        ref[n, pl.ds(r, 2 * tr), :] = val.astype(BF16)

    def st_wide(ref, blk, val, nsl, tr=T2):
        for n in range(nsl):
            stp(ref, n, blk, val[:, n * 128:(n + 1) * 128], tr)

    def ld_wide(ref, blk, nsl, tr=T2):
        return _cat([ldp(ref, n, blk, tr) for n in range(nsl)])

    def w_wide(vm, lo, hi):
        return _cat([ldw(vm, n) for n in range(lo, hi)])

    def x_blk(i):
        r = i * T
        if not isinstance(i, int):
            r = pl.multiple_of(r, T)
        return x_v[pl.ds(r, T), :].astype(F32)

    XW = {1: (2, 3), 2: tuple(range(4, NB))} if NB == 8 else {1: (2,), 2: (3,)}
    x_copy(0).start()
    if SV == 1:
        x_copy(1).start()
    start(wk_c)
    start(b_c)
    if SV == 3:
        x_copy(1).start()

    def bias_table():
        for i in range(S // 128):
            row = b_v[pl.ds(i, 1), :].astype(F32) * (1.0 / GS)
            bb_v[pl.ds(i * 128, 128), :] = jnp.broadcast_to(row, (128, 128)).T

    xs_refs = (xn0, xn1)
    hn_refs = (hn0, hn1)
    zt_refs = (zt0, zt1)

    def a_ops(ref, blk, he, ho, cr):
        a11, a12, a21, a22 = he[:, :256], he[:, 256:], ho[:, :256], ho[:, 256:]
        ops = (a11 + a22, a21 + a22, a11, a22, a11 + a12, a21 - a11, a12 - a22, a12, a21)
        for m, op in enumerate(ops):
            for n in range(2):
                stp(ref, 2 * m + n, blk, op[:, n * 128:(n + 1) * 128], cr // 2)

    def a_ld(ref, blk):
        def aop(m):
            return _cat([ldp(ref, 2 * m + n, blk, 64) for n in range(2)])
        return aop

    def a_full(aop):
        return jnp.concatenate([_cat([aop(2), aop(7)]), _cat([aop(8), aop(3)])], axis=0)

    def w_ops(src, b, nh, dst, d0, n):
        for h in range(WC):
            hr = 256 // WC
            w11, w12, w21, w22 = [ldw(src, b + nh * q + n, 256 * p + h * hr, hr).astype(F32)
                                  for p in range(2) for q in range(2)]
            for j, op in enumerate((w11 + w22, w12 - w22, w21 - w11, w11 + w12, w21 + w22)):
                dst[d0 + nh * j + n, pl.ds(h * hr, hr), :] = op.astype(BF16)

    def w_jit(src, b, nh, dst, d0, n):
        w11, w12, w21, w22 = [ldw(src, b + nh * q + n, 256 * p, 256) for p in range(2) for q in range(2)]
        f11, f12, f21, f22 = [w.astype(F32) for w in (w11, w12, w21, w22)]
        cs = [op.astype(BF16) for op in (f11 + f22, f12 - f22, f21 - f11, f11 + f12, f21 + f22)]
        for j, op in enumerate(cs):
            dst[d0 + nh * j + n] = op
        ops = (cs[0], w11, cs[1], cs[2], w22, cs[3], cs[4])
        return lambda m, n_: ops[m]

    def w_get(src, b, nh, dst, d0, n, jit):
        return w_jit(src, b, nh, dst, d0, n) if jit else functools.partial(w_op, src, b, nh, dst, d0)

    def w_op(src, b, nh, dst, d0, m, n):
        if m == 1:
            return ldw(src, b + n, 0, 256)
        if m == 4:
            return ldw(src, b + nh + n, 256, 256)
        return ldw(dst, d0 + nh * {0: 0, 2: 1, 3: 2, 5: 3, 6: 4}[m] + n)

    def strassen(aop, wop, order, put, n, nh):
        pr = {m: _dot(aop(m), wop(m, n)) for m in order}
        put(0, n, pr[0] + pr[3] - pr[4] + pr[6])
        put(0, nh + n, pr[2] + pr[4])
        put(1, n, pr[1] + pr[3])
        put(1, nh + n, pr[0] - pr[1] + pr[2] + pr[5])

    def phi_proj(i, b, d0, fast, jit):
        aop = a_ld(xs_refs[i % 2], i // 2)
        if not fast:
            return _phi(_dot(a_full(aop), w_wide(wqkv_v, b, b + 4)))
        out = {}

        def put(p, n, c):
            out[p, n] = _phi(c)
        for n in range(2):
            strassen(aop, w_get(wqkv_v, b, 2, wqs_v, d0, n, jit), QORD, put, n, 2)
        return jnp.concatenate([_cat([out[p, n] for n in range(4)]) for p in range(2)], axis=0)

    def ln_x(i, par):
        cr = 128 // NCX
        for c in range(NCX):
            he = _ln(x_v[pl.ds(i * T + c * cr, cr), :].astype(F32), D)
            ho = _ln(x_v[pl.ds(i * T + 128 + c * cr, cr), :].astype(F32), D)
            a_ops(xs_refs[par], (i // 2) * NCX + c, he, ho, cr)

    def ka(i):
        pk = phi_proj(i, 4, 0, i >= KS, i == KS)
        xn = a_full(a_ld(xs_refs[i % 2], i // 2))
        zsum = jnp.sum(pk.reshape(T // 8, 8, D), axis=0)
        a = lax.dot_general(pk.astype(BF16), xn, TN, preferred_element_type=F32)
        if i == 0:
            zs_v[...] = zsum
            a_v[...] = a
        else:
            zs_v[...] += zsum
            a_v[...] += a

    with jax.named_scope("phase1"):
        x_copy(0).wait()
        for b in ((1,) if SV in (0, 2) else ()) + XW[1]:
            x_copy(b).start()
        ln_x(0, 0)
        wait(wk_c)
        if SV != 2:
            x_copy(1).wait()
        for b in XW[2]:
            x_copy(b).start()
        for i in range(NB):
            for b in XW.get(i, ()):
                x_copy(b).wait()
            if i == 1:
                start(wq_c)
                start(wv_c)
                start(wo_c)
            if i == 2:
                start(win_c)
                start(wout_c)
                wait(b_c)
                bias_table()
            ka(i)
            if i + 1 < NB:
                ln_x(i + 1, (i + 1) % 2)

    start(wsp_c)

    def q_proj(i):
        return phi_proj(i, 0, 10, i >= QS, i == QS)

    def rr_part(i, pq):
        pqb = pq.astype(BF16)
        for g in range(4):
            pg = pqb[:, g * 128:(g + 1) * 128]
            den = _dot(pg, ldw(zbd_v, g))
            stp(pq_v, g, i, (pq[:, g * 128:(g + 1) * 128] if RF else pg.astype(F32)) * pl.reciprocal(den + 1e-6, approx=True))

    def attn_part(i, par, defer=False):
        hf = x_blk(i) + _dot(ld_wide(pq_v, i, 4), w_wide(m_v, 0, 4))
        st_wide(h_v, i, hf, 4)

        def ln_chunk(c, nc):
            cr = 128 // nc
            he = _ln(hf[c * cr:(c + 1) * cr], D, 1.0, GA)
            ho = _ln(hf[128 + c * cr:128 + (c + 1) * cr], D, 1.0, GA)
            a_ops(hn_refs[par], c, he, ho, cr)
        if defer:
            return [functools.partial(ln_chunk, c, NCH) for c in range(NCH)]
        ln_chunk(0, 1)

    def wout_ops(ns, which):
        for n in ns:
            for h in which:
                w11, w12, w21, w22 = [ldw(wout_v, 2 * q + n, 384 * p + h * 128, 128).astype(F32)
                                      for p in range(2) for q in range(2)]
                for m, op in ((0, w11 + w22), (2, w12 - w22), (3, w21 - w11), (5, w11 + w12), (6, w21 + w22)):
                    wos_v[2 * m + n, pl.ds(h * 128, 128), :] = op.astype(BF16)

    def wout_jit(n):
        w11, w12, w21, w22 = [ldw(wout_v, 2 * q + n, 384 * p, 384) for p in range(2) for q in range(2)]
        f11, f12, f21, f22 = [w.astype(F32) for w in (w11, w12, w21, w22)]
        return [w if w.dtype == BF16 else w.astype(BF16) for w in
                (f11 + f22, w11, f12 - f22, f21 - f11, w22, f11 + f12, f21 + f22)]

    def wout_op(m, n):
        if m == 1:
            return ldw(wout_v, n, 0, 384)
        if m == 4:
            return ldw(wout_v, 2 + n, 384, 384)
        return ldw(wos_v, 2 * m + n)

    def win_ops(part, ns):
        for n in ns:
            w_ops(win_v, 7 * part, 3, wis_v, 15 * part, n)

    with jax.named_scope("phase1b"):
        wait(wq_c)
        wait(wv_c)
        wait(wo_c)
        wait(wout_c)
        wait(win_c)
        same = (lax.broadcasted_iota(jnp.int32, (128, 128), 0) // DH
                == lax.broadcasted_iota(jnp.int32, (128, 128), 1) // DH)
        zrow = jnp.sum(zs_v[...], axis=0, keepdims=True)
        for g in range(4):
            zcol = jnp.broadcast_to(zrow[:, g * 128:(g + 1) * 128], (128, 128)).T
            zbd_v[g] = jnp.where(same, zcol, 0.0).astype(BF16)
        pq = q_proj(0)
        kvs = [_dot(a_v[pl.ds(g * 128, 128), :].astype(BF16), ldw(wqkv_v, 8 + g)) for g in range(4)]
        pq1 = q_proj(1)
        rr_part(0, pq)
        for g in range(4):
            kvb = jnp.where(same, kvs[g], 0.0).astype(BF16)
            mg = _dot(kvb, _cat([ldw(wo_v, n, g * 128, 128) for n in range(4)]))
            for n in range(4):
                m_v[n, pl.ds(g * 128, 128), :] = mg[:, n * 128:(n + 1) * 128].astype(BF16)
        pq = pq1
        for i in range(2, NB):
            pqn = q_proj(i)
            rr_part(i - 1, pq)
            pq = pqn
            if i == 2:
                attn_part(0, 0)
        rr_part(NB - 1, pq)

    def pair(i, par, has_next, jit=False):
        aop = a_ld(hn_refs[par], 0)

        def e_tile(part, n, put):
            if n == 3:
                c = _dot(a_full(aop), ldw(win_v, 7 * part + 6))
                put(0, 6, c[:128]); put(1, 6, c[128:])
            else:
                strassen(aop, w_get(win_v, 7 * part, 3, wis_v, 15 * part, n, jit), EORD, put, n, 3)

        zt = zt_refs[par]

        def put2(p, n, c):
            zt[p * 128:(p + 1) * 128, n * 128:(n + 1) * 128] = _gelu2(c)

        def put1(p, n, c):
            stp(z1_v, n, 2 * i + p, _gelu2(c), 64)
        for n in range(4):
            e_tile(1, n, put2)
        todo = []
        if has_next:
            todo += attn_part(i + 1, 1 - par, True)

        def lnz(c):
            cr = 128 // NCZ
            ze = _ln(zt[c * cr:(c + 1) * cr, :], FH, GS, 1.0 / GS)
            zo = _ln(zt[128 + c * cr:128 + (c + 1) * cr, :], FH, GS, 1.0 / GS)
            b11, b12, b21, b22 = ze[:, :384], ze[:, 384:768], zo[:, :384], zo[:, 384:768]
            ops = (b11 + b22, b11, b12 - b22, b21 - b11, b22, b11 + b12, b21 + b22)
            for m, op in enumerate(ops):
                for n in range(3):
                    stp(z2_v, 3 * m + n, i * NCZ + c, op[:, n * 128:(n + 1) * 128], cr // 2)
            stp(z7_v, 0, (2 * i) * NCZ + c, ze[:, 768:], cr // 2)
            stp(z7_v, 0, (2 * i + 1) * NCZ + c, zo[:, 768:], cr // 2)
        todo += [functools.partial(lnz, c) for c in range(NCZ)]
        for n in range(4):
            e_tile(0, n, put1)
            k = -(-len(todo) // (4 - n)) if ORD == 0 else (len(todo) if n >= min(ORD, 3) else 0)
            for f in todo[:k]:
                f()
            todo = todo[k:]

    def p2(j, c):
        pair(2 * j + 1, 1, True)
        pair(2 * j + 2, 0, True)
        return c

    with jax.named_scope("phase2"):
        pair(0, 0, True, True)
        lax.fori_loop(0, NB // 2 - 1, p2, 0)
        pair(NB - 1, 1, False)

    wait(wsp_c)

    R3 = T3 // 2

    def p3(i, carry):
        r = i * T3 if isinstance(i, int) else pl.multiple_of(i * T3, T3)
        def wsl(k, half):
            v = wsp_v.at[k].bitcast(U32)
            if half is None:
                return pltpu.bitcast(v[pl.ds(mo(i * R3, R3), R3), :], BF16)
            return pltpu.bitcast(v[pl.ds(mo(i * R3 + half * (R3 // 2), R3 // 2), R3 // 2), :], BF16)

        def a_blk(p, q):
            return _cat([wsl(2 * k + q, p) for k in range(8)])

        def a_sum(p, q, p2, q2, sign):
            a = _cat([wsl(2 * k + q, p).astype(F32) for k in range(8)])
            b = _cat([wsl(2 * k + q2, p2).astype(F32) for k in range(8)])
            return (a + b if sign > 0 else a - b).astype(BF16)

        def b_op(m):
            return w_wide(z2_v, 3 * m, 3 * m + 3)

        g7 = _dot(_cat([wsl(k, None) for k in range(16)]), ldw(z7_v, 0))
        m1 = _dot(a_sum(0, 0, 1, 1, 1), b_op(0))
        m2 = _dot(a_sum(1, 0, 1, 1, 1), b_op(1))
        m3 = _dot(a_blk(0, 0), b_op(2))
        m4 = _dot(a_blk(1, 1), b_op(3))
        m5 = _dot(a_sum(0, 0, 0, 1, 1), b_op(4))
        m6 = _dot(a_sum(1, 0, 0, 0, -1), b_op(5))
        m7 = _dot(a_sum(0, 1, 1, 1, -1), b_op(6))
        c11 = m1 + m4 - m5 + m7
        c12 = m3 + m5
        c21 = m2 + m4
        c22 = m1 - m2 + m3 + m6
        TH = T3 // 2

        def gate(c, p, n0):
            nt = c.shape[1] // 128
            bb = bb_v[pl.ds(r + p * TH, TH), :]
            z1 = _cat([ldp(z1_v, n0 + n, 2 * i + p, TH // 2) for n in range(nt)]).astype(F32)
            return z1 * (c + _cat([bb] * nt))
        y11, y12, y21, y22 = gate(c11, 0, 0), gate(c12, 0, 3), gate(c21, 1, 0), gate(c22, 1, 3)
        y7 = jnp.concatenate([gate(g7[:TH], 0, 6), gate(g7[TH:], 1, 6)], axis=0).astype(BF16)
        lhs = ((y11 + y22).astype(BF16), (y21 + y22).astype(BF16), y11.astype(BF16), y22.astype(BF16),
               (y11 + y12).astype(BF16), (y21 - y11).astype(BF16), (y12 - y22).astype(BF16))
        for n in range(2):
            o7 = [_dot(y7, ldw(wout_v, 2 * q + n, 768, 128)) + ldp(h_v, 2 * q + n, i, R3).astype(F32) for q in range(2)]
            wops = wout_jit(n) if WO == 3 else [wout_op(m, n) for m in range(7)]
            pr = {m: _dot(lhs[m], wops[m]) for m in GORD}
            n1, n2, n3, n4, n5, n6, n7 = [pr[m] for m in range(7)]
            outs = ((o7[0][:TH] + n1 + n4 - n5 + n7, o7[1][:TH] + n3 + n5),
                    (o7[0][TH:] + n2 + n4, o7[1][TH:] + n1 - n2 + n3 + n6))
            for q in range(2):
                for p in range(2):
                    o_v[2 * q + n, pl.ds(r + p * TH, TH), :] = outs[p][q].astype(BF16)
                o_copy(i, 2 * q + n).start()
        return carry

    with jax.named_scope("phase3"):
        if U3:
            for i in range(N3):
                p3(i, 0)
        else:
            lax.fori_loop(0, N3, p3, 0)

    for i in range(N3):
        for n in range(4):
            o_copy(i, n).wait()


def make(T=256, T3=512, NCH=2, NCZ=4, ORD=0, FL=0, SV=1, WO=3, GO=2, U2=0, U3=0, EO=2, WC=8, RF=0, KS=2, QS=0, QO=2, NCX=1):
    flags = {0: None, 1: {'XLA_TPU_FORCE_LP_LLO_SCHEDULER': True}, 2: {'XLA_TPU_EVENLY_DISTRIBUTE_CRITICAL_NODES': True}, 3: {'XLA_TPU_FORCE_LP_LLO_SCHEDULER': True, 'XLA_TPU_EVENLY_DISTRIBUTE_CRITICAL_NODES': True}, 4: {'XLA_TPU_RESCHEDULE_DMA_DONES': True}}[FL]
    @jax.jit
    def fn(A_x, A_wqkv, A_wo, B_x, B_w_in, B_w_sp, B_b_sp, B_w_out):
        del B_x
        any_spec = pl.BlockSpec(memory_space=pl.ANY)
        return pl.pallas_call(
            functools.partial(_kernel, T=T, T3=T3, NCH=NCH, NCZ=NCZ, ORD=ORD, SV=SV, WO=WO, GO=GO, U2=U2, U3=U3, EO=EO, WC=WC, RF=RF, KS=KS, QS=QS, QO=QO, NCX=NCX),
            in_specs=[any_spec] * 7,
            out_specs=any_spec,
            out_shape=jax.ShapeDtypeStruct((1, S, D), BF16),
            scratch_shapes=[
                pltpu.VMEM((S, D), BF16),
                pltpu.VMEM((12, D, 128), BF16),
                pltpu.VMEM((4, D, 128), BF16),
                pltpu.VMEM((14, D, 128), BF16),
                pltpu.VMEM((16, S, 128), BF16),
                pltpu.VMEM((S // 128, 128), BF16),
                pltpu.VMEM((4, FH, 128), BF16),
                pltpu.VMEM((18, S // 4, 128), BF16),
                pltpu.VMEM((18, S // 4, 128), BF16),
                pltpu.VMEM((4, S, 128), BF16),
                pltpu.VMEM((D, D), F32),
                pltpu.VMEM((8, D), F32),
                pltpu.VMEM((4, D, 128), BF16),
                pltpu.VMEM((4, 128, 128), BF16),
                pltpu.VMEM((S, 128), F32),
                pltpu.VMEM((4, S, 128), BF16),
                pltpu.VMEM((18, 128, 128), BF16),
                pltpu.VMEM((18, 128, 128), BF16),
                pltpu.VMEM((7, S, 128), BF16),
                pltpu.VMEM((21, S // 2, 128), BF16),
                pltpu.VMEM((1, S, 128), BF16),
                pltpu.VMEM((14, 384, 128), BF16),
                pltpu.VMEM((30, 256, 128), BF16),
                pltpu.VMEM((20, 256, 128), BF16),
                pltpu.VMEM((4, S, 128), BF16),
                pltpu.VMEM((T, FH), F32),
                pltpu.VMEM((T, FH), F32),
                pltpu.SemaphoreType.DMA((S // T,)),
                pltpu.SemaphoreType.DMA((7,)),
                pltpu.SemaphoreType.DMA((1,)),
                pltpu.SemaphoreType.DMA((S // T3,)),
            ],
            compiler_params=pltpu.CompilerParams(vmem_limit_bytes=100 * 1024 * 1024, flags=flags),
        )(A_x, A_wqkv, A_wo, B_w_in, B_w_sp, B_b_sp.reshape(S // 128, 128), B_w_out)
    return fn


_fn = make()


def pallas_sequential_preLN__linear_attn_block__mixer_gmlp__prompt_kernel(
        A_x, A_wqkv, A_wo, B_x, B_w_in, B_w_sp, B_b_sp, B_w_out):
    return _fn(A_x, A_wqkv, A_wo, B_x, B_w_in, B_w_sp, B_b_sp, B_w_out)
```

```python
import functools
import jax
import jax.numpy as jnp
from jax import lax
from jax.experimental import pallas as pl
from jax.experimental.pallas import tpu as pltpu

S, D, H, DH, FH = 2048, 512, 32, 16, 896
LN_EPS = 1e-5
F32, BF16, U32 = jnp.float32, jnp.bfloat16, jnp.uint32
GC1 = 0.7978845608028654
GC2 = GC1 * 0.044715
GA = GC2 ** (1.0 / 3.0)
GK = GC1 / GA
GS = 2.0 * GA
TN = (((0,), (0,)), ((), ()))
T, T3 = 256, 512
NCH, NCZ = 2, 4
KS = 2
QORD = EORD = GORD = (3, 1, 4, 6, 0, 2, 5)
AORD = (6, 0, 3, 4, 2, 1, 5)
FORD = (7, 6, 0, 3, 4, 2, 1, 5)


def _dot(a, b):
    return jnp.dot(a, b, preferred_element_type=F32)


def _ln(xf, n, s_in=1.0, s_out=1.0):
    m = jnp.sum(xf, axis=-1, keepdims=True) * (1.0 / n)
    xc = xf - m
    v = jnp.sum(xc * xc, axis=-1, keepdims=True) * (1.0 / (n * s_out * s_out))
    return xc * jnp.exp2(-0.5 * jnp.log2(v + LN_EPS * (s_in / s_out) ** 2))


def _phi(t):
    return (jnp.maximum(t, 0.0) + jnp.exp(jnp.minimum(t, 0.0))) + 1e-6


def _gelu2(t):
    return t + t * jnp.tanh(t * (t * t + GK))


def _cat(xs):
    return xs[0] if len(xs) == 1 else jnp.concatenate(xs, axis=1)


def _kernel(x_hbm, wqkv_hbm, wo_hbm, win_hbm, wsp_hbm, b_hbm, wout_hbm, out_hbm,
            x_v, wqkv_v, wo_v, win_v, wsp_v, b_v, wout_v,
            xn0, xn1, pq_v, a_v, zs_v, m_v, zbd_v, bb_v, h_v, hn0, hn1, z1_v, z2_v, z7_v, wis_v, wqs_v, ms_v, o_v, zt0, zt1,
            sem_x, sem_w, sem_sp, sem_o):
    NB, N3 = S // T, S // T3
    T2 = T // 2

    def x_copy(i):
        return pltpu.make_async_copy(x_hbm.at[0, pl.ds(i * T, T)], x_v.at[pl.ds(i * T, T)], sem_x.at[i])

    def slab_copies(hbm, vm, lo, hi, sem):
        return [pltpu.make_async_copy(hbm.at[:, pl.ds(n * 128, 128)], vm.at[n], sem) for n in range(lo, hi)]

    def o_copy(i, n):
        return pltpu.make_async_copy(o_v.at[n, pl.ds(i * T3, T3)],
                                     out_hbm.at[0, pl.ds(i * T3, T3), pl.ds(n * 128, 128)], sem_o.at[i])

    wk_c = slab_copies(wqkv_hbm, wqkv_v, 4, 8, sem_w.at[0])
    wq_c = slab_copies(wqkv_hbm, wqkv_v, 0, 4, sem_w.at[1])
    wv_c = slab_copies(wqkv_hbm, wqkv_v, 8, 12, sem_w.at[2])
    wo_c = slab_copies(wo_hbm, wo_v, 0, 4, sem_w.at[3])
    win_c = slab_copies(win_hbm, win_v, 0, 14, sem_w.at[4])
    wout_c = slab_copies(wout_hbm, wout_v, 0, 4, sem_w.at[5])
    wsp_c = slab_copies(wsp_hbm, wsp_v, 0, 16, sem_sp.at[0])
    b_c = [pltpu.make_async_copy(b_hbm, b_v, sem_w.at[6])]

    def start(cs):
        for c in cs:
            c.start()

    def wait(cs):
        for c in cs:
            c.wait()

    def ldw(vm, n, r0=0, nr=None):
        v = vm.at[n].bitcast(U32)
        nr = v.shape[0] * 2 if nr is None else nr
        return pltpu.bitcast(v[pl.ds(r0 // 2, nr // 2), :], BF16)

    def ldp(ref, n, blk, tr=T2):
        r = blk * tr
        if not isinstance(blk, int):
            r = pl.multiple_of(r, tr)
        return pltpu.bitcast(ref.at[n].bitcast(U32)[pl.ds(r, tr), :], BF16)

    def stp(ref, n, blk, val, tr=T2):
        r = blk * (2 * tr)
        if not isinstance(blk, int):
            r = pl.multiple_of(r, 2 * tr)
        ref[n, pl.ds(r, 2 * tr), :] = val.astype(BF16)

    def st_wide(ref, blk, val, nsl, tr=T2):
        for n in range(nsl):
            stp(ref, n, blk, val[:, n * 128:(n + 1) * 128], tr)

    def w_wide(vm, lo, hi):
        return _cat([ldw(vm, n) for n in range(lo, hi)])

    def x_blk(i):
        r = i * T
        if not isinstance(i, int):
            r = pl.multiple_of(r, T)
        return x_v[pl.ds(r, T), :].astype(F32)

    XW = {1: (2, 3), 2: tuple(range(4, NB))}
    x_copy(0).start()
    x_copy(1).start()
    start(wk_c)
    start(b_c)

    def bias_table():
        for i in range(S // 128):
            row = b_v[pl.ds(i, 1), :].astype(F32) * (1.0 / GS)
            bb_v[pl.ds(i * 128, 128), :] = jnp.broadcast_to(row, (128, 128)).T

    xs_refs = (xn0, xn1)
    hn_refs = (hn0, hn1)
    zt_refs = (zt0, zt1)

    def a_ops(ref, blk, he, ho, cr, nops):
        a11, a12, a21, a22 = he[:, :256], he[:, 256:], ho[:, :256], ho[:, 256:]
        ops = (a11 + a22, a21 + a22, a11, a22, a11 + a12, a21 - a11, a12 - a22, a12, a21)
        for m, op in enumerate(ops[:nops]):
            for n in range(2):
                stp(ref, 2 * m + n, blk, op[:, n * 128:(n + 1) * 128], cr // 2)

    def a_ld(ref, blk):
        def aop(m):
            return _cat([ldp(ref, 2 * m + n, blk, 64) for n in range(2)])
        return aop

    def a_full(aop):
        return jnp.concatenate([_cat([aop(2), aop(7)]), _cat([aop(8), aop(3)])], axis=0)

    def w_get(src, s0, s1, dst, d, jit):
        if jit:
            w11, w12, w21, w22 = [ldw(src, sl, 256 * p, 256) for p in range(2) for sl in (s0, s1)]
            f11, f12, f21, f22 = [w.astype(F32) for w in (w11, w12, w21, w22)]
            cs = [op.astype(BF16) for op in (f11 + f22, f12 - f22, f21 - f11, f11 + f12, f21 + f22)]
            for j, op in enumerate(cs):
                dst[d + j] = op
            ops = (cs[0], w11, cs[1], cs[2], w22, cs[3], cs[4])
            return lambda m: ops[m]

        def wop(m):
            if m == 1:
                return ldw(src, s0, 0, 256)
            if m == 4:
                return ldw(src, s1, 256, 256)
            return ldw(dst, d + {0: 0, 2: 1, 3: 2, 5: 3, 6: 4}[m])
        return wop

    def strassen(aop, wop, order, put0, put1):
        pr = {m: _dot(aop(m), wop(m)) for m in order}
        put0(0, pr[0] + pr[3] - pr[4] + pr[6])
        put1(0, pr[2] + pr[4])
        put0(1, pr[1] + pr[3])
        put1(1, pr[0] - pr[1] + pr[2] + pr[5])

    def phi_proj(i, b, d0, fast, jit):
        aop = a_ld(xs_refs[i % 2], i // 2)
        if not fast:
            return _phi(_dot(a_full(aop), w_wide(wqkv_v, b, b + 4)))
        out = {}

        def put(n, p, c):
            out[p, n] = _phi(c)
        for n in range(2):
            strassen(aop, w_get(wqkv_v, b + n, b + 2 + n, wqs_v, d0 + 5 * n, jit), QORD,
                     functools.partial(put, n), functools.partial(put, 2 + n))
        return jnp.concatenate([_cat([out[p, n] for n in range(4)]) for p in range(2)], axis=0)

    def ln_x(i, par):
        he = _ln(x_v[pl.ds(i * T, 128), :].astype(F32), D)
        ho = _ln(x_v[pl.ds(i * T + 128, 128), :].astype(F32), D)
        a_ops(xs_refs[par], i // 2, he, ho, 128, 9)

    def ka(i):
        pk = phi_proj(i, 4, 0, i >= KS, i == KS)
        xn = a_full(a_ld(xs_refs[i % 2], i // 2))
        zsum = jnp.sum(pk.reshape(T // 8, 8, D), axis=0)
        a = lax.dot_general(pk.astype(BF16), xn, TN, preferred_element_type=F32)
        if i == 0:
            zs_v[...] = zsum
            a_v[...] = a
        else:
            zs_v[...] += zsum
            a_v[...] += a

    x_copy(0).wait()
    for b in XW[1]:
        x_copy(b).start()
    ln_x(0, 0)
    wait(wk_c)
    x_copy(1).wait()
    for b in XW[2]:
        x_copy(b).start()
    for i in range(NB):
        for b in XW.get(i, ()):
            x_copy(b).wait()
        if i == 1:
            start(wq_c)
            start(wv_c)
            start(wo_c)
        if i == 2:
            start(win_c)
            start(wout_c)
            wait(b_c)
            bias_table()
        ka(i)
        if i + 1 < NB:
            ln_x(i + 1, (i + 1) % 2)

    start(wsp_c)

    def q_proj(i):
        return phi_proj(i, 0, 10, True, i == 0)

    def rr_part(i, pq):
        pqb = pq.astype(BF16)
        rs = []
        for g in range(4):
            pg = pqb[:, g * 128:(g + 1) * 128]
            den = _dot(pg, ldw(zbd_v, g))
            rs.append(pg.astype(F32) * pl.reciprocal(den + 1e-6, approx=True))
        rr = _cat(rs)
        a_ops(pq_v, i, rr[:128], rr[128:], 128, 7)

    def attn_mm(i, jit):
        xb = x_blk(i)
        out = {}

        def put(n, p, c):
            out[p, n] = xb[p * 128:(p + 1) * 128, n * 128:(n + 1) * 128] + c
        for n in range(2):
            strassen(a_ld(pq_v, i), w_get(m_v, n, 2 + n, ms_v, 5 * n, jit), AORD,
                     functools.partial(put, n), functools.partial(put, 2 + n))
        return jnp.concatenate([_cat([out[p, n] for n in range(4)]) for p in range(2)], axis=0)

    def attn_part(i, par, defer=False):
        hf = attn_mm(i, isinstance(i, int) and i == 0)
        st_wide(h_v, i, hf, 4)

        def ln_chunk(c, nc):
            cr = 128 // nc
            he = _ln(hf[c * cr:(c + 1) * cr], D, 1.0, GA)
            ho = _ln(hf[128 + c * cr:128 + (c + 1) * cr], D, 1.0, GA)
            a_ops(hn_refs[par], c, he, ho, cr, 7)
        if defer:
            return [functools.partial(ln_chunk, c, NCH) for c in range(NCH)]
        ln_chunk(0, 1)

    def wout_jit(n):
        w11, w12, w21, w22 = [ldw(wout_v, 2 * q + n, 384 * p, 384) for p in range(2) for q in range(2)]
        f11, f12, f21, f22 = [w.astype(F32) for w in (w11, w12, w21, w22)]
        return [w if w.dtype == BF16 else w.astype(BF16) for w in
                (f11 + f22, w11, f12 - f22, f21 - f11, w22, f11 + f12, f21 + f22)]

    wait(wq_c)
    wait(wv_c)
    wait(wo_c)
    wait(wout_c)
    wait(win_c)
    same = (lax.broadcasted_iota(jnp.int32, (128, 128), 0) // DH
            == lax.broadcasted_iota(jnp.int32, (128, 128), 1) // DH)
    zrow = jnp.sum(zs_v[...], axis=0, keepdims=True)
    for g in range(4):
        zcol = jnp.broadcast_to(zrow[:, g * 128:(g + 1) * 128], (128, 128)).T
        zbd_v[g] = jnp.where(same, zcol, 0.0).astype(BF16)
    pq = q_proj(0)
    kvs = [_dot(a_v[pl.ds(g * 128, 128), :].astype(BF16), ldw(wqkv_v, 8 + g)) for g in range(4)]
    pq1 = q_proj(1)
    rr_part(0, pq)
    for g in range(4):
        kvb = jnp.where(same, kvs[g], 0.0).astype(BF16)
        mg = _dot(kvb, _cat([ldw(wo_v, n, g * 128, 128) for n in range(4)]))
        for n in range(4):
            m_v[n, pl.ds(g * 128, 128), :] = mg[:, n * 128:(n + 1) * 128].astype(BF16)
    pq = pq1
    for i in range(2, NB):
        pqn = q_proj(i)
        rr_part(i - 1, pq)
        pq = pqn
        if i == 2:
            attn_part(0, 0)
    rr_part(NB - 1, pq)

    def pair(i, par, has_next, jit=False):
        aop = a_ld(hn_refs[par], 0)

        def e_group(g):
            (s0, p0, n0), (s1, p1, n1) = (((7 + g, put2, g), (10 + g, put2, 3 + g)) if g < 3 else
                                          ((13, put2, 6), (6, put1, 6)) if g == 3 else
                                          ((g - 4, put1, g - 4), (g - 1, put1, g - 1)))
            strassen(aop, w_get(win_v, s0, s1, wis_v, 5 * g, jit), EORD,
                     functools.partial(p0, n0), functools.partial(p1, n1))

        zt = zt_refs[par]

        def put2(n, p, c):
            zt[p * 128:(p + 1) * 128, n * 128:(n + 1) * 128] = _gelu2(c)

        def put1(n, p, c):
            stp(z1_v, n, 2 * i + p, _gelu2(c), 64)
        for n in range(4):
            e_group(n)
        todo = []
        if has_next:
            todo += attn_part(i + 1, 1 - par, True)

        def lnz(c):
            cr = 128 // NCZ
            ze = _ln(zt[c * cr:(c + 1) * cr, :], FH, GS, 1.0 / GS)
            zo = _ln(zt[128 + c * cr:128 + (c + 1) * cr, :], FH, GS, 1.0 / GS)
            b11, b12, b21, b22 = ze[:, :384], ze[:, 384:768], zo[:, :384], zo[:, 384:768]
            ops = (b11 + b22, b11, b12 - b22, b21 - b11, b22, b11 + b12, b21 + b22)
            for m, op in enumerate(ops):
                for n in range(3):
                    stp(z2_v, 3 * m + n, i * NCZ + c, op[:, n * 128:(n + 1) * 128], cr // 2)
            stp(z7_v, 0, (2 * i) * NCZ + c, ze[:, 768:], cr // 2)
            stp(z7_v, 0, (2 * i + 1) * NCZ + c, zo[:, 768:], cr // 2)
        todo += [functools.partial(lnz, c) for c in range(NCZ)]
        for n in range(3):
            e_group(4 + n)
            k = -(-len(todo) // (3 - n))
            for f in todo[:k]:
                f()
            todo = todo[k:]

    def p2(j, c):
        pair(2 * j + 1, 1, True)
        pair(2 * j + 2, 0, True)
        return c

    pair(0, 0, True, True)
    lax.fori_loop(0, NB // 2 - 1, p2, 0)
    pair(NB - 1, 1, False)

    wait(wsp_c)

    R3 = T3 // 2

    def p3(i, carry):
        r = pl.multiple_of(i * T3, T3)

        def wsl(k, half):
            v = wsp_v.at[k].bitcast(U32)
            if half is None:
                return pltpu.bitcast(v[pl.ds(pl.multiple_of(i * R3, R3), R3), :], BF16)
            return pltpu.bitcast(v[pl.ds(pl.multiple_of(i * R3 + half * (R3 // 2), R3 // 2), R3 // 2), :], BF16)

        def a_blk(p, q):
            return _cat([wsl(2 * k + q, p) for k in range(8)])

        def a_sum(p, q, p2, q2, sign):
            a = _cat([wsl(2 * k + q, p).astype(F32) for k in range(8)])
            b = _cat([wsl(2 * k + q2, p2).astype(F32) for k in range(8)])
            return (a + b if sign > 0 else a - b).astype(BF16)

        def b_op(m):
            return w_wide(z2_v, 3 * m, 3 * m + 3)

        fs = (lambda: _dot(a_sum(0, 0, 1, 1, 1), b_op(0)), lambda: _dot(a_sum(1, 0, 1, 1, 1), b_op(1)),
              lambda: _dot(a_blk(0, 0), b_op(2)), lambda: _dot(a_blk(1, 1), b_op(3)),
              lambda: _dot(a_sum(0, 0, 0, 1, 1), b_op(4)), lambda: _dot(a_sum(1, 0, 0, 0, -1), b_op(5)),
              lambda: _dot(a_sum(0, 1, 1, 1, -1), b_op(6)),
              lambda: _dot(_cat([wsl(k, None) for k in range(16)]), ldw(z7_v, 0)))
        pf = {m: fs[m]() for m in FORD}
        m1, m2, m3, m4, m5, m6, m7, g7 = [pf[m] for m in range(8)]
        c11 = m1 + m4 - m5 + m7
        c12 = m3 + m5
        c21 = m2 + m4
        c22 = m1 - m2 + m3 + m6
        TH = T3 // 2

        def gate(c, p, n0):
            nt = c.shape[1] // 128
            bb = bb_v[pl.ds(r + p * TH, TH), :]
            z1 = _cat([ldp(z1_v, n0 + n, 2 * i + p, TH // 2) for n in range(nt)]).astype(F32)
            return z1 * (c + _cat([bb] * nt))
        y11, y12, y21, y22 = gate(c11, 0, 0), gate(c12, 0, 3), gate(c21, 1, 0), gate(c22, 1, 3)
        y7 = jnp.concatenate([gate(g7[:TH], 0, 6), gate(g7[TH:], 1, 6)], axis=0).astype(BF16)
        lhs = ((y11 + y22).astype(BF16), (y21 + y22).astype(BF16), y11.astype(BF16), y22.astype(BF16),
               (y11 + y12).astype(BF16), (y21 - y11).astype(BF16), (y12 - y22).astype(BF16))
        for n in range(2):
            o7 = [_dot(y7, ldw(wout_v, 2 * q + n, 768, 128)) + ldp(h_v, 2 * q + n, i, R3).astype(F32) for q in range(2)]
            wops = wout_jit(n)
            pr = {m: _dot(lhs[m], wops[m]) for m in GORD}
            n1, n2, n3, n4, n5, n6, n7 = [pr[m] for m in range(7)]
            outs = ((o7[0][:TH] + n1 + n4 - n5 + n7, o7[1][:TH] + n3 + n5),
                    (o7[0][TH:] + n2 + n4, o7[1][TH:] + n1 - n2 + n3 + n6))
            for q in range(2):
                for p in range(2):
                    o_v[2 * q + n, pl.ds(r + p * TH, TH), :] = outs[p][q].astype(BF16)
                o_copy(i, 2 * q + n).start()
        return carry

    lax.fori_loop(0, N3, p3, 0)

    for i in range(N3):
        for n in range(4):
            o_copy(i, n).wait()


@jax.jit
def pallas_sequential_preLN__linear_attn_block__mixer_gmlp__prompt_kernel(
    A_x: jax.Array,
    A_wqkv: jax.Array,
    A_wo: jax.Array,
    B_x: jax.Array,
    B_w_in: jax.Array,
    B_w_sp: jax.Array,
    B_b_sp: jax.Array,
    B_w_out: jax.Array,
):
    del B_x
    any_spec = pl.BlockSpec(memory_space=pl.ANY)
    return pl.pallas_call(
        _kernel,
        in_specs=[any_spec] * 7,
        out_specs=any_spec,
        out_shape=jax.ShapeDtypeStruct((1, S, D), BF16),
        scratch_shapes=[
            pltpu.VMEM((S, D), BF16),
            pltpu.VMEM((12, D, 128), BF16),
            pltpu.VMEM((4, D, 128), BF16),
            pltpu.VMEM((14, D, 128), BF16),
            pltpu.VMEM((16, S, 128), BF16),
            pltpu.VMEM((S // 128, 128), BF16),
            pltpu.VMEM((4, FH, 128), BF16),
            pltpu.VMEM((18, S // 4, 128), BF16),
            pltpu.VMEM((18, S // 4, 128), BF16),
            pltpu.VMEM((14, S // 2, 128), BF16),
            pltpu.VMEM((D, D), F32),
            pltpu.VMEM((8, D), F32),
            pltpu.VMEM((4, D, 128), BF16),
            pltpu.VMEM((4, 128, 128), BF16),
            pltpu.VMEM((S, 128), F32),
            pltpu.VMEM((4, S, 128), BF16),
            pltpu.VMEM((14, 128, 128), BF16),
            pltpu.VMEM((14, 128, 128), BF16),
            pltpu.VMEM((7, S, 128), BF16),
            pltpu.VMEM((21, S // 2, 128), BF16),
            pltpu.VMEM((1, S, 128), BF16),
            pltpu.VMEM((35, 256, 128), BF16),
            pltpu.VMEM((20, 256, 128), BF16),
            pltpu.VMEM((10, 256, 128), BF16),
            pltpu.VMEM((4, S, 128), BF16),
            pltpu.VMEM((T, FH), F32),
            pltpu.VMEM((T, FH), F32),
            pltpu.SemaphoreType.DMA((S // T,)),
            pltpu.SemaphoreType.DMA((7,)),
            pltpu.SemaphoreType.DMA((1,)),
            pltpu.SemaphoreType.DMA((S // T3,)),
        ],
        compiler_params=pltpu.CompilerParams(vmem_limit_bytes=100 * 1024 * 1024),
    )(A_x, A_wqkv, A_wo, B_w_in, B_w_sp, B_b_sp.reshape(S // 128, 128), B_w_out)
```
